```python
import os as _os
_os.environ.setdefault("JAX_PLATFORMS", "cpu")
import jax
import jax.numpy as jnp

def _softmax(x, axis=-1):
    return jax.nn.softmax(x, axis=axis)
def _gelu(x):
    return jax.nn.gelu(x, approximate=True)
def _silu(x):
    return jax.nn.silu(x)
def _sigmoid(x):
    return jax.nn.sigmoid(x)
def _layernorm(x, axis=-1, eps=1e-5):
    m = jnp.mean(x, axis=axis, keepdims=True)
    v = jnp.var(x, axis=axis, keepdims=True)
    return (x - m) / jnp.sqrt(v + eps)
def _scatter_add(tgt, idx, src, axis=0):
    return tgt.at[idx].add(src)
def _segment_sum(src, seg, n):
    return jax.ops.segment_sum(src, seg, n)
class _Rng:
    def __init__(self, key):
        self._k = key
    def _next(self):
        self._k, sub = jax.random.split(self._k)
        return sub
    def normal(self, shape):
        return jax.random.normal(self._next(), shape, dtype=jnp.bfloat16)
    def randint(self, lo, hi, shape):
        return jax.random.randint(self._next(), shape, lo, hi, dtype=jnp.int32)
    def uniform(self, shape, lo=0.0, hi=1.0):
        return jax.random.uniform(self._next(), shape, jnp.bfloat16, lo, hi)
    def permutation(self, n):
        return jax.random.permutation(self._next(), n)


kernel_name = 'concat_heads__mha_block_cached__gqa_block_cached__decode'

def setup_inputs():
    _rng = _Rng(jax.random.key(int.from_bytes(__import__("os").urandom(4), "little")))
    _w = (lambda a: (lambda t: t.astype(jnp.bfloat16) if jnp.issubdtype(t.dtype, jnp.floating) else t)(jnp.asarray(a)))
    def _A_setup():
        B, Sq, D = 1, 1, 512
        H, Sk, Dh = 32, 4096, 128
        return {
            "x": _w((lambda *s: _rng.normal(s) * 0.8)(B, Sq, D)),
            "k_cache": _w((lambda *s: _rng.normal(s) * 0.8)(B, H, Sk, Dh)),
            "v_cache": _w((lambda *s: _rng.normal(s) * 0.05)(B, H, Sk, Dh)),
            "wq": _w((lambda *s: _rng.normal(s) * 0.8)(D, H * Dh) * (D ** -0.5)),
            "wo": _w((lambda *s: _rng.normal(s) * 0.05)(H * Dh, D) * ((H * Dh) ** -0.5)),
        }
    _A_in = _A_setup()

    def _B_setup():
        B, Sq, D = 1, 1, 512
        Hq, Hkv, Sk, Dh = 32, 32, 4096, 128
        assert Hq % Hkv == 0, (Hq, Hkv)
        return {
            "x": _w((lambda *s: _rng.normal(s) * 0.8)(B, Sq, D)),
            "k_cache": _w((lambda *s: _rng.normal(s) * 0.8)(B, Hkv, Sk, Dh)),
            "v_cache": _w((lambda *s: _rng.normal(s) * 0.05)(B, Hkv, Sk, Dh)),
            "wq": _w((lambda *s: _rng.normal(s) * 0.8)(D, Hq * Dh) * (D ** -0.5)),
            "wo": _w((lambda *s: _rng.normal(s) * 0.05)(Hq * Dh, D) * ((Hq * Dh) ** -0.5)),
        }
    _B_in = _B_setup()

    return {
        "A_x": _A_in["x"],
        "A_k_cache": _A_in["k_cache"],
        "A_v_cache": _A_in["v_cache"],
        "A_wq": _A_in["wq"],
        "A_wo": _A_in["wo"],
        "B_x": _B_in["x"],
        "B_k_cache": _B_in["k_cache"],
        "B_v_cache": _B_in["v_cache"],
        "B_wq": _B_in["wq"],
        "B_wo": _B_in["wo"],
    }

def reference(A_x, A_k_cache, A_v_cache, A_wq, A_wo, B_x, B_k_cache, B_v_cache, B_wq, B_wo):
    def _A_ref(x, k_cache, v_cache, wq, wo):
        B, Sq, D = x.shape
        H, Dh = 32, 128
        q = (lambda x, *d: x.transpose(*d))((x @ wq).reshape(B, Sq, H, Dh), 0, 2, 1, 3)
        scores = jnp.einsum("bhqd,bhkd->bhqk", q, k_cache) * (Dh ** -0.5)
        p = _softmax(scores, axis=-1)
        o = jnp.einsum("bhqk,bhkd->bhqd", p, v_cache)
        return (lambda x, *d: x.transpose(*d))(o, 0, 2, 1, 3).reshape(B, Sq, H * Dh) @ wo

    def _B_ref(x, k_cache, v_cache, wq, wo):
        B, Sq, D = x.shape
        Hq, Dh = 32, 128
        Hkv = k_cache.shape[1]
        rep = Hq // Hkv
        q = (lambda x, *d: x.transpose(*d))((x @ wq).reshape(B, Sq, Hq, Dh), 0, 2, 1, 3)
        k = jnp.repeat(k_cache, rep, axis=1)
        v = jnp.repeat(v_cache, rep, axis=1)
        scores = jnp.einsum("bhqd,bhkd->bhqk", q, k) * (Dh ** -0.5)
        p = _softmax(scores, axis=-1)
        o = jnp.einsum("bhqk,bhkd->bhqd", p, v)
        return (lambda x, *d: x.transpose(*d))(o, 0, 2, 1, 3).reshape(B, Sq, Hq * Dh) @ wo

    a = _A_ref(A_x, A_k_cache, A_v_cache, A_wq, A_wo)
    b = _B_ref(B_x, B_k_cache, B_v_cache, B_wq, B_wo)
    return jnp.concatenate([a, b], axis=-1)
```

```python
import jax
import jax.numpy as jnp
from jax import lax
import jax.experimental.pallas as pl
import jax.experimental.pallas.tpu as pltpu

_D = 512
_H = 32
_SK = 4096
_DH = 128
_T = 128
_NG = _SK // _T
_AHEAD = 2
_SLOTS = _AHEAD + 1
_NQ = 4
_NO = 16

_NT = (((1,), (1,)), ((), ()))


def _bit_reverse(i, bits):
    return int(format(i, "0%db" % bits)[::-1], 2)


def _kernel(ax, ak, av, awq, awo, bx, bk, bv, bwq, bwo, out_ref,
            x_buf, wq_buf, ring, wo_buf, q_buf, s_buf,
            x_sem, wq_sem, ring_sem, wo_sem):
    xs, ks, vs, wqs, wos = (ax, bx), (ak, bk), (av, bv), (awq, bwq), (awo, bwo)
    f32, bf16 = jnp.float32, jnp.bfloat16
    row = lax.broadcasted_iota(jnp.int32, (8, _DH), 0)

    def start_wq(c):
        cols = pl.ds(pl.multiple_of(c * 1024, 1024), 1024)
        for i in range(32):
            rows = pl.ds(_bit_reverse(i, 5) * 16, 16)
            for b in range(2):
                pltpu.make_async_copy(
                    wqs[b].at[rows, cols], wq_buf.at[c, b, rows], wq_sem.at[c]
                ).start(priority=b)

    def start_slab(srcs, g, slot):
        rows = pl.ds(pl.multiple_of(g * (_T // 2), _T // 2), _T // 2)
        for h in range(_H):
            for b in range(2):
                pltpu.make_async_copy(
                    srcs[b].at[pl.ds(2 * h, 2), rows],
                    ring.at[slot, pl.ds(2 * (b * _H + h), 2)],
                    ring_sem.at[slot],
                ).start(priority=b)

    def start_wo(j):
        for i in range(8):
            for u in range(4):
                r = u * 4 + j
                src_rows = pl.ds(pl.multiple_of(r * _DH + i * 16, 16), 16)
                for b in range(2):
                    pltpu.make_async_copy(
                        wos[b].at[:, src_rows],
                        wo_buf.at[r, b, :, pl.ds(i * 16, 16)],
                        wo_sem.at[r],
                    ).start(priority=b)

    def wait_all(buf, sem):
        pltpu.make_async_copy(buf, buf, sem).wait()

    def next_slot(slot):
        return jnp.where(slot == _SLOTS - 1, 0, slot + 1)

    def prev_slot(slot):
        return jnp.where(slot == 0, _SLOTS - 1, slot - 1)

    def tile(slot, i):
        return ring[slot, pl.ds(2 * i, 2)].reshape(_T, _DH)

    def own_rows(parts):
        res = parts[0]
        for r in range(1, 8):
            res = jnp.where(row == r, parts[r], res)
        return res

    @pl.loop(0, _AHEAD)
    def _(c):
        start_wq(c)

    x_copies = [pltpu.make_async_copy(xs[b], x_buf.at[b], x_sem.at[b]) for b in range(2)]
    for cp in x_copies:
        cp.start()
    for cp in x_copies:
        cp.wait()

    @pl.loop(0, _NQ)
    def _(c):
        @pl.when(c + _AHEAD < _NQ)
        def _():
            start_wq(c + _AHEAD)

        @pl.when(c + _AHEAD >= _NQ)
        def _():
            start_slab(ks, c + _AHEAD - _NQ, c + _AHEAD - _NQ)

        wait_all(wq_buf.at[c], wq_sem.at[c])
        for b in range(2):
            x8 = jnp.broadcast_to(x_buf[b, 0].astype(f32), (8, _D)).astype(bf16)
            q = jnp.dot(x8, wq_buf[c, b], preferred_element_type=f32)
            q_buf[b * _NQ + c] = own_rows(
                [q[:, r * _DH:(r + 1) * _DH] for r in range(8)])

    nrow = 2 * _H // 8
    scale = _DH ** -0.5

    def k_step(g, carry):
        slot, ms = carry

        @pl.when(g + _AHEAD < _NG)
        def _():
            start_slab(ks, g + _AHEAD, prev_slot(slot))

        @pl.when(g + _AHEAD >= _NG)
        def _():
            start_slab(vs, g + _AHEAD - _NG, prev_slot(slot))

        wait_all(ring.at[slot], ring_sem.at[slot])
        new_ms = []
        for j in range(nrow):
            q8 = q_buf[j].astype(bf16)
            s = own_rows([
                lax.dot_general(q8, tile(slot, 8 * j + r), _NT,
                                preferred_element_type=f32)
                for r in range(8)]) * scale
            s_buf[g, j] = s
            new_ms.append(jnp.maximum(ms[j], s))
        return next_slot(slot), tuple(new_ms)

    neg_inf = jnp.full((8, _T), -jnp.inf, f32)
    slot, ms = lax.fori_loop(0, _NG, k_step, (0, (neg_inf,) * nrow))
    ms = [jnp.broadcast_to(jnp.max(m, axis=1, keepdims=True), (8, _T)) for m in ms]

    def v_step(g, carry):
        slot, ls, accs = carry

        @pl.when(g + _AHEAD < _NG)
        def _():
            start_slab(vs, g + _AHEAD, prev_slot(slot))

        @pl.when(g + _AHEAD >= _NG)
        def _():
            start_wo(g + _AHEAD - _NG)

        wait_all(ring.at[slot], ring_sem.at[slot])
        new_ls, new_accs = [], []
        for j in range(nrow):
            p = jnp.exp(s_buf[g, j] - ms[j])
            p8 = p.astype(bf16)
            o = own_rows([
                jnp.dot(p8, tile(slot, 8 * j + r), preferred_element_type=f32)
                for r in range(8)])
            new_ls.append(ls[j] + p)
            new_accs.append(accs[j] + o)
        return next_slot(slot), tuple(new_ls), tuple(new_accs)

    zero = jnp.zeros((8, _DH), f32)
    _, ls, accs = lax.fori_loop(0, _NG, v_step, (slot, (zero,) * nrow, (zero,) * nrow))
    for j in range(nrow):
        q_buf[j] = accs[j] / jnp.sum(ls[j], axis=1, keepdims=True)

    def o_step(j, outs):
        @pl.when(j + _AHEAD < 4)
        def _():
            start_wo(j + _AHEAD)

        outs = list(outs)
        for u in range(4):
            r = u * 4 + j
            wait_all(wo_buf.at[r], wo_sem.at[r])
            for b in range(2):
                for half in range(2):
                    h = half * 16 + u * 4
                    o = q_buf[b * _NQ + h // 8, pl.ds(h % 8 + j, 1), :]
                    o8 = jnp.broadcast_to(o, (8, _DH)).astype(bf16)
                    outs[b] = outs[b] + jnp.dot(
                        o8, wo_buf[r, b, half], preferred_element_type=f32)
        return tuple(outs)

    zero = jnp.zeros((8, _D), f32)
    outs = lax.fori_loop(0, 4, o_step, (zero, zero))
    out_ref[0] = jnp.concatenate([o[0:1] for o in outs], axis=1).astype(out_ref.dtype)


@jax.jit
def pallas_concat_heads__mha_block_cached__gqa_block_cached__decode_kernel(
    A_x: jax.Array,
    A_k_cache: jax.Array,
    A_v_cache: jax.Array,
    A_wq: jax.Array,
    A_wo: jax.Array,
    B_x: jax.Array,
    B_k_cache: jax.Array,
    B_v_cache: jax.Array,
    B_wq: jax.Array,
    B_wo: jax.Array,
):
    bf16 = jnp.bfloat16

    def halves(cache):
        assert cache.shape == (1, _H, _SK, _DH), cache.shape
        return cache.reshape(2 * _H, _SK // 2, _DH)

    def wo_halves(wo):
        return wo.reshape(2, _H * _DH // 2, _D)

    return pl.pallas_call(
        _kernel,
        in_specs=[pl.BlockSpec(memory_space=pltpu.HBM)] * 10,
        out_specs=pl.BlockSpec(memory_space=pltpu.VMEM),
        out_shape=jax.ShapeDtypeStruct((1, 1, 2 * _D), A_x.dtype),
        scratch_shapes=[
            pltpu.VMEM((2, 1, 1, _D), bf16),
            pltpu.VMEM((_NQ, 2, _D, 1024), bf16),
            pltpu.VMEM((_SLOTS, 4 * _H, _T // 2, _DH), bf16),
            pltpu.VMEM((_NO, 2, 2, _DH, _D), bf16),
            pltpu.VMEM((2 * _H // 8, 8, _DH), jnp.float32),
            pltpu.VMEM((_NG, 2 * _H // 8, 8, _T), jnp.float32),
            pltpu.SemaphoreType.DMA((2,)),
            pltpu.SemaphoreType.DMA((_NQ,)),
            pltpu.SemaphoreType.DMA((_SLOTS,)),
            pltpu.SemaphoreType.DMA((_NO,)),
        ],
        compiler_params=pltpu.CompilerParams(vmem_limit_bytes=64 * 1024 * 1024),
    )(A_x, halves(A_k_cache), halves(A_v_cache), A_wq, wo_halves(A_wo),
      B_x, halves(B_k_cache), halves(B_v_cache), B_wq, wo_halves(B_wo))
```

```python
import functools

import jax
import jax.numpy as jnp
from jax import lax
import jax.experimental.pallas as pl
import jax.experimental.pallas.tpu as pltpu

_D = 512
_H = 32
_SK = 4096
_DH = 128
_G = 8
_NJ = _H // _G
_P = 64
_T = 512
_NC = _SK // _T
_AHEAD = 2
_SLOTS = _AHEAD + 1
_NU = 32
_NU_SLAB = _T // _P
_PREFILL = 30
_LEAD = 8
_DELAY = 3

_NT = (((1,), (1,)), ((), ()))


def _own_rows(parts):
    row = lax.broadcasted_iota(jnp.int32, parts[0].shape, 0)
    res = parts[0]
    for r in range(1, _G):
        res = jnp.where(row == r, parts[r], res)
    return res


def _fold_lanes(op, v):
    return functools.reduce(op, [v[:, i:i + 128] for i in range(0, v.shape[1], 128)])


def _wait_filled(buf, sem):
    pltpu.make_async_copy(buf, buf, sem).wait()


def _body(ax, ak, av, awq, awo, bx, bk, bv, bwq, bwo, out_ref,
          x_buf, wq_buf, ring, wo_buf, s_buf, o_buf, acc_buf,
          x_sem, wq_sem, ring_sem, wo_sem):
    xs, ks, vs, wqs, wos = (ax, bx), (ak, bk), (av, bv), (awq, bwq), (awo, bwo)
    f32, bf16 = jnp.float32, jnp.bfloat16
    group_cols = _G * _DH

    def start_wq(i, prefill=0):
        n = 0
        for half in range(2):
            rows = pl.ds(pl.multiple_of(i * 16 + half * 8, 8), 8)
            for j in range(_NJ):
                for pair in range(2):
                    for b in range(2):
                        pltpu.make_async_copy(
                            wqs[b].at[:, pair, rows, pl.ds(j * group_cols, group_cols)],
                            wq_buf.at[b, j, :, pair, rows],
                            wq_sem,
                        ).start(priority=1 if n < prefill else b)
                        n += 1

    def start_slab(srcs, j, c, slot):
        for i in range(_T // _P):
            rows = pl.ds(pl.multiple_of(c * _T + i * _P, _P), _P)
            for h in range(0, _G, 2):
                for b in range(2):
                    pltpu.make_async_copy(
                        srcs[b].at[pl.ds(j * _G + h, 2), rows],
                        ring.at[slot, b, pl.ds(h, 2), pl.ds(i * _P, _P)],
                        ring_sem.at[slot],
                    ).start(priority=b)

    def start_wo(n):
        for i in range(2):
            rows = pl.ds(pl.multiple_of(n * 32 + i * 16, 16), 16)
            for pair in range(2):
                for b in range(2):
                    pltpu.make_async_copy(
                        wos[b].at[:, pair, rows],
                        wo_buf.at[b, n, :, pl.ds(pair * 32 + i * 16, 16)],
                        wo_sem.at[b, n],
                    ).start(priority=b)

    def next_slot(slot):
        return jnp.where(slot == _SLOTS - 1, 0, slot + 1)

    def prev_slot(slot):
        return jnp.where(slot == 0, _SLOTS - 1, slot - 1)

    start_wq(0, _PREFILL)
    x_copies = [pltpu.make_async_copy(xs[b], x_buf.at[b], x_sem.at[b]) for b in range(2)]
    for b, cp in enumerate(x_copies):
        cp.start(priority=b)

    @pl.loop(1, _D // 4 // 16)
    def _(i):
        start_wq(i)

    @pl.loop(0, _AHEAD)
    def _(c):
        start_slab(ks, 0, c, c)

    for cp in x_copies:
        cp.wait()
    _wait_filled(wq_buf, wq_sem)

    def head_group(j, slot):
        qs = []
        for b in range(2):
            x = jnp.broadcast_to(x_buf[b, 0].astype(f32), (_G, _D)).astype(bf16)
            w = jnp.concatenate([wq_buf[b, j, u // 2, u % 2] for u in range(4)], axis=0)
            q = jnp.dot(x, w, preferred_element_type=f32)
            qs.append(_own_rows([q[:, r * _DH:(r + 1) * _DH] for r in range(_G)]).astype(bf16))

        def k_step(c, carry):
            slot, ms = carry

            @pl.when(c + _AHEAD < _NC)
            def _():
                start_slab(ks, j, c + _AHEAD, prev_slot(slot))

            @pl.when(c + _AHEAD >= _NC)
            def _():
                start_slab(vs, j, c + _AHEAD - _NC, prev_slot(slot))

            _wait_filled(ring.at[slot], ring_sem.at[slot])
            new_ms = []
            for b in range(2):
                s = _own_rows([
                    lax.dot_general(qs[b], ring[slot, b, r], _NT, preferred_element_type=f32)
                    for r in range(_G)]) * (_DH ** -0.5)
                s_buf[c, b] = s
                new_ms.append(jnp.maximum(ms[b], _fold_lanes(jnp.maximum, s)))
            return next_slot(slot), tuple(new_ms)

        neg_inf = jnp.full((_G, 128), -jnp.inf, f32)
        slot, ms = lax.fori_loop(0, _NC, k_step, (slot, (neg_inf, neg_inf)))
        ms = [jnp.max(m, axis=1, keepdims=True) for m in ms]

        def v_step(c, carry):
            slot, ls, accs = carry

            @pl.when(c + _AHEAD < _NC)
            def _():
                start_slab(vs, j, c + _AHEAD, prev_slot(slot))

            @pl.when(c + _AHEAD >= _NC)
            def _():
                @pl.when(j < _NJ - 1)
                def _():
                    start_slab(ks, j + 1, c + _AHEAD - _NC, prev_slot(slot))

                @pl.when(j == _NJ - 1)
                def _():
                    @pl.loop(0, _NU_SLAB)
                    def _(u):
                        start_wo((c + _AHEAD - _NC) * _NU_SLAB + u)

            _wait_filled(ring.at[slot], ring_sem.at[slot])
            new_ls, new_accs = [], []
            for b in range(2):
                p = jnp.exp(s_buf[c, b] - ms[b])
                p16 = p.astype(bf16)
                o = _own_rows([
                    jnp.dot(p16, ring[slot, b, r], preferred_element_type=f32)
                    for r in range(_G)])
                new_ls.append(ls[b] + _fold_lanes(jnp.add, p))
                new_accs.append(accs[b] + o)
            return next_slot(slot), tuple(new_ls), tuple(new_accs)

        zero = jnp.zeros((_G, _DH), f32)
        slot, ls, accs = lax.fori_loop(0, _NC, v_step, (slot, (zero, zero), (zero, zero)))
        for b in range(2):
            o_buf[b, j] = accs[b] / jnp.sum(ls[b], axis=1, keepdims=True)
        return slot

    lax.fori_loop(0, _NJ, head_group, 0)

    for b in range(2):
        groups = [o_buf[b, j] for j in range(_NJ)]
        for c in range(4):
            o_buf[b, c] = jnp.concatenate([o[:, 32 * c:32 * c + 32] for o in groups], axis=1)
    acc_buf[...] = jnp.zeros(acc_buf.shape, f32)

    @pl.loop(0, 2 * _NU)
    def _(t):
        started = _AHEAD * _NU_SLAB
        nxt = (t >> 1) + started - _DELAY

        @pl.when(((t & 1) == 1) & (nxt >= started) & (nxt < _NU))
        def _():
            start_wo(nxt)

        m = t - _LEAD
        head, tail = m < 0, t >= 2 * _NU - _LEAD
        b = jnp.where(head, 0, jnp.where(tail, 1, 1 - (m & 1)))
        n = jnp.where(head, t, jnp.where(tail, t - _NU, (m >> 1) + _LEAD * (m & 1)))
        o = jnp.broadcast_to(o_buf[b, n & 3, pl.ds(n >> 2, 1), :], (_G, _DH)).astype(bf16)
        _wait_filled(wo_buf.at[b, n], wo_sem.at[b, n])
        w = jnp.concatenate([wo_buf[b, n, 0], wo_buf[b, n, 1]], axis=0)
        acc_buf[b] += jnp.dot(o, w, preferred_element_type=f32)

    out = jnp.concatenate([acc_buf[b, 0:1] for b in range(2)], axis=1)
    out_ref[0] = out.astype(out_ref.dtype)


def _kernel(*refs):
    pl.run_scoped(
        functools.partial(_body, *refs),
        pltpu.SemaphoreType.DMA((2,)),
        pltpu.SemaphoreType.DMA,
        pltpu.SemaphoreType.DMA((_SLOTS,)),
        pltpu.SemaphoreType.DMA((2, _NU)),
    )


@jax.jit
def pallas_concat_heads__mha_block_cached__gqa_block_cached__decode_kernel(
    A_x: jax.Array,
    A_k_cache: jax.Array,
    A_v_cache: jax.Array,
    A_wq: jax.Array,
    A_wo: jax.Array,
    B_x: jax.Array,
    B_k_cache: jax.Array,
    B_v_cache: jax.Array,
    B_wq: jax.Array,
    B_wo: jax.Array,
):
    f32, bf16 = jnp.float32, jnp.bfloat16

    def heads(cache):
        return cache.reshape(_H, _SK, _DH)

    def quarters(w):
        return w.reshape(2, 2, w.shape[0] // 4, w.shape[1])

    return pl.pallas_call(
        _kernel,
        in_specs=[pl.BlockSpec(memory_space=pltpu.HBM)] * 10,
        out_specs=pl.BlockSpec(memory_space=pltpu.VMEM),
        out_shape=jax.ShapeDtypeStruct((1, 1, 2 * _D), A_x.dtype),
        scratch_shapes=[
            pltpu.VMEM((2, 1, 1, _D), bf16),
            pltpu.VMEM((2, _NJ, 2, 2, _D // 4, _G * _DH), bf16),
            pltpu.VMEM((_SLOTS, 2, _G, _T, _DH), bf16),
            pltpu.VMEM((2, _NU, 2, 64, _D), bf16),
            pltpu.VMEM((_NC, 2, _G, _T), f32),
            pltpu.VMEM((2, _NJ, _G, _DH), f32),
            pltpu.VMEM((2, _G, _D), f32),
        ],
        compiler_params=pltpu.CompilerParams(vmem_limit_bytes=48 * 1024 * 1024),
    )(A_x, heads(A_k_cache), heads(A_v_cache), quarters(A_wq), quarters(A_wo),
      B_x, heads(B_k_cache), heads(B_v_cache), quarters(B_wq), quarters(B_wo))
```

```python
import functools

import jax
import jax.numpy as jnp
from jax import lax
import jax.experimental.pallas as pl
import jax.experimental.pallas.tpu as pltpu

_D = 512
_H = 32
_SK = 4096
_DH = 128
_G = 8
_NJ = _H // _G
_P = 64
_T = 512
_NC = _SK // _T
_AHEAD = 2
_SLOTS = _AHEAD + 1
_NU = 32
_NU_SLAB = _T // _P
_PREFILL = 30
_LEAD = 8
_SKEW = 3

_NT = (((1,), (1,)), ((), ()))


def _own_rows(parts):
    row = lax.broadcasted_iota(jnp.int32, parts[0].shape, 0)
    res = parts[0]
    for r in range(1, _G):
        res = jnp.where(row == r, parts[r], res)
    return res


def _fold_lanes(op, v):
    return functools.reduce(op, [v[:, i:i + 128] for i in range(0, v.shape[1], 128)])


def _wait_filled(buf, sem):
    pltpu.make_async_copy(buf, buf, sem).wait()


def _body(ax, ak, av, awq, awo, bx, bk, bv, bwq, bwo, out_ref,
          x_buf, wq_buf, ring, wo_buf, s_buf, o_buf, col_buf,
          x_sem, wq_sem, ring_sem, wo_sem):
    xs, ks, vs, wqs, wos = (ax, bx), (ak, bk), (av, bv), (awq, bwq), (awo, bwo)
    f32, bf16 = jnp.float32, jnp.bfloat16
    group_cols = _G * _DH

    def start_wq(i, prefill=0):
        n = 0
        for half in range(2):
            rows = pl.ds(pl.multiple_of(i * 16 + half * 8, 8), 8)
            for j in range(_NJ):
                for pair in range(2):
                    for b in range(2):
                        pltpu.make_async_copy(
                            wqs[b].at[:, pair, rows, pl.ds(j * group_cols, group_cols)],
                            wq_buf.at[b, j, :, pair, rows],
                            wq_sem,
                        ).start(priority=1 if n < prefill else b)
                        n += 1

    def start_slab(srcs, j, c, slot):
        first_keys = (c * _T, ((c + _SKEW) & (_NC - 1)) * _T)
        for i in range(_T // _P):
            for h in range(0, _G, 2):
                for b in range(2):
                    rows = pl.ds(pl.multiple_of(first_keys[b] + i * _P, _P), _P)
                    pltpu.make_async_copy(
                        srcs[b].at[pl.ds(j * _G + h, 2), rows],
                        ring.at[slot, b, pl.ds(h, 2), pl.ds(i * _P, _P)],
                        ring_sem.at[slot],
                    ).start(priority=b)

    def wo_copy(b, n, k):
        i, pair = divmod(k, 2)
        rows = pl.ds(pl.multiple_of(n * 32 + i * 16, 16), 16)
        sem = b * _NU + n
        if b == 1:
            sem = jnp.where(n < _NU - _LEAD, sem, sem + k * _LEAD)
        return pltpu.make_async_copy(
            wos[b].at[:, pair, rows],
            wo_buf.at[b, n, :, pl.ds(pair * 32 + i * 16, 16)],
            wo_sem.at[sem])

    def start_wo(n):
        for k in range(4):
            for b in range(2):
                wo_copy(b, n, k).start(priority=b)

    def next_slot(slot):
        return jnp.where(slot == _SLOTS - 1, 0, slot + 1)

    def prev_slot(slot):
        return jnp.where(slot == 0, _SLOTS - 1, slot - 1)

    start_wq(0, _PREFILL)
    x_copies = [pltpu.make_async_copy(xs[b], x_buf.at[b], x_sem.at[b]) for b in range(2)]
    for b, cp in enumerate(x_copies):
        cp.start(priority=b)

    @pl.loop(1, _D // 4 // 16)
    def _(i):
        start_wq(i)

    @pl.loop(0, _AHEAD)
    def _(c):
        start_slab(ks, 0, c, c)

    for cp in x_copies:
        cp.wait()
    _wait_filled(wq_buf, wq_sem)

    def head_group(j, slot):
        qs = []
        for b in range(2):
            x = jnp.broadcast_to(x_buf[b, 0].astype(f32), (_G, _D)).astype(bf16)
            w = jnp.concatenate([wq_buf[b, j, u // 2, u % 2] for u in range(4)], axis=0)
            q = jnp.dot(x, w, preferred_element_type=f32)
            qs.append(_own_rows([q[:, r * _DH:(r + 1) * _DH] for r in range(_G)]).astype(bf16))

        def k_step(c, carry):
            slot, ms = carry

            @pl.when(c + _AHEAD < _NC)
            def _():
                start_slab(ks, j, c + _AHEAD, prev_slot(slot))

            @pl.when(c + _AHEAD >= _NC)
            def _():
                start_slab(vs, j, c + _AHEAD - _NC, prev_slot(slot))

            _wait_filled(ring.at[slot], ring_sem.at[slot])
            new_ms = []
            for b in range(2):
                s = _own_rows([
                    lax.dot_general(qs[b], ring[slot, b, r], _NT, preferred_element_type=f32)
                    for r in range(_G)]) * (_DH ** -0.5)
                s_buf[c, b] = s
                new_ms.append(jnp.maximum(ms[b], _fold_lanes(jnp.maximum, s)))
            return next_slot(slot), tuple(new_ms)

        neg_inf = jnp.full((_G, 128), -jnp.inf, f32)
        slot, ms = lax.fori_loop(0, _NC, k_step, (slot, (neg_inf, neg_inf)))
        ms = [jnp.max(m, axis=1, keepdims=True) for m in ms]

        def v_step(c, carry):
            slot, ls, accs = carry

            @pl.when(c + _AHEAD < _NC)
            def _():
                start_slab(vs, j, c + _AHEAD, prev_slot(slot))

            @pl.when(c + _AHEAD >= _NC)
            def _():
                @pl.when(j < _NJ - 1)
                def _():
                    start_slab(ks, j + 1, c + _AHEAD - _NC, prev_slot(slot))

                @pl.when(j == _NJ - 1)
                def _():
                    @pl.loop(0, _NU_SLAB)
                    def _(u):
                        start_wo((c + _AHEAD - _NC) * _NU_SLAB + u)

            _wait_filled(ring.at[slot], ring_sem.at[slot])
            new_ls, new_accs = [], []
            for b in range(2):
                p = jnp.exp(s_buf[c, b] - ms[b])
                p16 = p.astype(bf16)
                o = _own_rows([
                    jnp.dot(p16, ring[slot, b, r], preferred_element_type=f32)
                    for r in range(_G)])
                new_ls.append(ls[b] + _fold_lanes(jnp.add, p))
                new_accs.append(accs[b] + o)
            return next_slot(slot), tuple(new_ls), tuple(new_accs)

        zero = jnp.zeros((_G, _DH), f32)
        slot, ls, accs = lax.fori_loop(0, _NC, v_step, (slot, (zero, zero), (zero, zero)))
        for b in range(2):
            o_buf[b, j] = accs[b] / jnp.sum(ls[b], axis=1, keepdims=True)
        return slot

    lax.fori_loop(0, _NJ, head_group, 0)

    for b in range(2):
        groups = [o_buf[b, j] for j in range(_NJ)]
        for c in range(4):
            o_buf[b, c] = jnp.concatenate([o[:, 32 * c:32 * c + 32] for o in groups], axis=1)

    def o_row(b, n):
        return o_buf[b, n & 3, pl.ds(n >> 2, 1), :]

    def wait_unit(b, n):
        _wait_filled(wo_buf.at[b, n], wo_sem.at[b * _NU + n])

    def unit(b, n):
        o = jnp.broadcast_to(o_row(b, n), (_G, _DH)).astype(bf16)
        w = jnp.concatenate([wo_buf[b, n, 0], wo_buf[b, n, 1]], axis=0)
        return jnp.dot(o, w, preferred_element_type=f32)

    def first_step(n, acc_a):
        o = o_row(1, n + _NU - _LEAD).astype(bf16).astype(f32)
        wait_unit(0, n)
        col_buf[n] = jnp.broadcast_to(o, (_DH, _DH)).T
        return acc_a + unit(0, n)

    def both_step(n, accs):
        @pl.when(n + _AHEAD * _NU_SLAB < _NU)
        def _():
            start_wo(n + _AHEAD * _NU_SLAB)

        wait_unit(0, n + _LEAD)
        wait_unit(1, n)
        return accs[0] + unit(0, n + _LEAD), accs[1] + unit(1, n)

    def last_step(v, acc):
        n = v + _NU - _LEAD
        for k in range(4):
            i, pair = divmod(k, 2)
            r0 = pair * 32 + i * 16
            wo_copy(1, n, k).wait()
            parts = []
            for half in range(2):
                col = jnp.tile(col_buf[v, pl.ds(half * 64 + r0, 16)], (1, _D // _DH))
                prod = wo_buf[1, n, half, pl.ds(r0, 16)].astype(f32) * col
                parts.append(prod[:8] + prod[8:])
            acc = acc + (parts[0] + parts[1])
        return acc

    zero = jnp.zeros((_G, _D), f32)
    acc_a = lax.fori_loop(0, _LEAD, first_step, zero)
    acc_a, acc_b = lax.fori_loop(0, _NU - _LEAD, both_step, (acc_a, zero))
    out_ref[0, :, pl.ds(0, _D)] = acc_a[0:1].astype(out_ref.dtype)
    acc_b = jnp.where(lax.broadcasted_iota(jnp.int32, (_G, _D), 0) == 0, acc_b, 0.0)
    acc_b = lax.fori_loop(0, _LEAD, last_step, acc_b)
    out_ref[0, :, pl.ds(_D, _D)] = jnp.sum(acc_b, axis=0, keepdims=True).astype(out_ref.dtype)


def _kernel(*refs):
    pl.run_scoped(
        functools.partial(_body, *refs),
        pltpu.SemaphoreType.DMA((2,)),
        pltpu.SemaphoreType.DMA,
        pltpu.SemaphoreType.DMA((_SLOTS,)),
        pltpu.SemaphoreType.DMA((2 * _NU + 3 * _LEAD,)),
    )


@jax.jit
def pallas_concat_heads__mha_block_cached__gqa_block_cached__decode_kernel(
    A_x: jax.Array,
    A_k_cache: jax.Array,
    A_v_cache: jax.Array,
    A_wq: jax.Array,
    A_wo: jax.Array,
    B_x: jax.Array,
    B_k_cache: jax.Array,
    B_v_cache: jax.Array,
    B_wq: jax.Array,
    B_wo: jax.Array,
):
    f32, bf16 = jnp.float32, jnp.bfloat16

    def heads(cache):
        return cache.reshape(_H, _SK, _DH)

    def quarters(w):
        return w.reshape(2, 2, w.shape[0] // 4, w.shape[1])

    return pl.pallas_call(
        _kernel,
        in_specs=[pl.BlockSpec(memory_space=pltpu.HBM)] * 10,
        out_specs=pl.BlockSpec(memory_space=pltpu.VMEM),
        out_shape=jax.ShapeDtypeStruct((1, 1, 2 * _D), A_x.dtype),
        scratch_shapes=[
            pltpu.VMEM((2, 1, 1, _D), bf16),
            pltpu.VMEM((2, _NJ, 2, 2, _D // 4, _G * _DH), bf16),
            pltpu.VMEM((_SLOTS, 2, _G, _T, _DH), bf16),
            pltpu.VMEM((2, _NU, 2, 64, _D), bf16),
            pltpu.VMEM((_NC, 2, _G, _T), f32),
            pltpu.VMEM((2, _NJ, _G, _DH), f32),
            pltpu.VMEM((_LEAD, _DH, _DH), f32),
        ],
        compiler_params=pltpu.CompilerParams(vmem_limit_bytes=48 * 1024 * 1024),
    )(A_x, heads(A_k_cache), heads(A_v_cache), quarters(A_wq), quarters(A_wo),
      B_x, heads(B_k_cache), heads(B_v_cache), quarters(B_wq), quarters(B_wo))
```

```python
import functools

import jax
import jax.numpy as jnp
from jax import lax
import jax.experimental.pallas as pl
import jax.experimental.pallas.tpu as pltpu

_D = 512
_H = 32
_SK = 4096
_DH = 128
_G = 8
_NJ = _H // _G
_P = 64
_T = 512
_NC = _SK // _T
_AHEAD = 2
_SLOTS = _AHEAD + 1
_SKEW = 3
_NU = 32
_NU_SLAB = _T // _P
_PREFILL = 30
_LEAD = 8

_NT = (((1,), (1,)), ((), ()))


def _own_rows(parts):
    row = lax.broadcasted_iota(jnp.int32, parts[0].shape, 0)
    res = parts[0]
    for r in range(1, _G):
        res = jnp.where(row == r, parts[r], res)
    return res


def _fold_lanes(op, v):
    return functools.reduce(op, [v[:, i:i + 128] for i in range(0, v.shape[1], 128)])


def _wait_filled(buf, sem):
    pltpu.make_async_copy(buf, buf, sem).wait()


def _body(ax, ak, av, awq, awo, bx, bk, bv, bwq, bwo, out_ref,
          x_buf, wq_buf, ring, wo_buf, s_buf, o_buf, col_buf,
          x_sem, wq_sem, ring_sem, wo_sem):
    xs, ks, vs, wqs, wos = (ax, bx), (ak, bk), (av, bv), (awq, bwq), (awo, bwo)
    f32, bf16 = jnp.float32, jnp.bfloat16
    group_cols = _G * _DH

    def start_wq(i, prefill=0):
        n = 0
        for half in range(2):
            rows = pl.ds(pl.multiple_of(i * 16 + half * 8, 8), 8)
            for j in range(_NJ):
                for pair in range(2):
                    for b in range(2):
                        pltpu.make_async_copy(
                            wqs[b].at[:, pair, rows, pl.ds(j * group_cols, group_cols)],
                            wq_buf.at[b, j, :, pair, rows],
                            wq_sem,
                        ).start(priority=1 if n < prefill else b)
                        n += 1

    def start_slab(srcs, j, c, slot):
        for i in range(_T // _P):
            keys = [(c * _T + (i + b * _SKEW) * _P) & (_SK - 1) for b in range(2)]
            rows = [pl.ds(pl.multiple_of(key, _P), _P) for key in keys]
            for h in range(0, _G, 2):
                for b in range(2):
                    pltpu.make_async_copy(
                        srcs[b].at[pl.ds(j * _G + h, 2), rows[b]],
                        ring.at[slot, b, pl.ds(h, 2), pl.ds(i * _P, _P)],
                        ring_sem.at[slot],
                    ).start(priority=b)

    def wo_rows(k):
        i, pair = divmod(k, 2)
        return pair * 32 + i * 16

    def wo_copy(b, n, k):
        i, pair = divmod(k, 2)
        rows = pl.ds(pl.multiple_of(n * 32 + i * 16, 16), 16)
        sem = b * _NU + n
        if b == 1:
            sem = jnp.where(n < _NU - _LEAD, sem, sem + k * _LEAD)
        return pltpu.make_async_copy(
            wos[b].at[:, pair, rows],
            wo_buf.at[b, n, :, pl.ds(wo_rows(k), 16)],
            wo_sem.at[sem])

    def start_wo(n):
        for k in range(4):
            for b in range(2):
                wo_copy(b, n, k).start(priority=b)

    def next_slot(slot):
        return jnp.where(slot == _SLOTS - 1, 0, slot + 1)

    def prev_slot(slot):
        return jnp.where(slot == 0, _SLOTS - 1, slot - 1)

    start_wq(0, _PREFILL)
    x_copies = [pltpu.make_async_copy(xs[b], x_buf.at[b], x_sem.at[b]) for b in range(2)]
    for b, cp in enumerate(x_copies):
        cp.start(priority=b)

    @pl.loop(1, _D // 4 // 16)
    def _(i):
        start_wq(i)

    @pl.loop(0, _AHEAD)
    def _(c):
        start_slab(ks, 0, c, c)

    for cp in x_copies:
        cp.wait()
    _wait_filled(wq_buf, wq_sem)

    def head_group(j, slot):
        qs = []
        for b in range(2):
            x = jnp.broadcast_to(x_buf[b, 0].astype(f32), (_G, _D)).astype(bf16)
            w = jnp.concatenate([wq_buf[b, j, u // 2, u % 2] for u in range(4)], axis=0)
            q = jnp.dot(x, w, preferred_element_type=f32)
            qs.append(_own_rows([q[:, r * _DH:(r + 1) * _DH] for r in range(_G)]).astype(bf16))

        def k_step(c, carry):
            slot, ms = carry

            @pl.when(c + _AHEAD < _NC)
            def _():
                start_slab(ks, j, c + _AHEAD, prev_slot(slot))

            @pl.when(c + _AHEAD >= _NC)
            def _():
                start_slab(vs, j, c + _AHEAD - _NC, prev_slot(slot))

            _wait_filled(ring.at[slot], ring_sem.at[slot])
            new_ms = []
            for b in range(2):
                s = _own_rows([
                    lax.dot_general(qs[b], ring[slot, b, r], _NT, preferred_element_type=f32)
                    for r in range(_G)]) * (_DH ** -0.5)
                s_buf[c, b] = s
                new_ms.append(jnp.maximum(ms[b], _fold_lanes(jnp.maximum, s)))
            return next_slot(slot), tuple(new_ms)

        neg_inf = jnp.full((_G, 128), -jnp.inf, f32)
        slot, ms = lax.fori_loop(0, _NC, k_step, (slot, (neg_inf, neg_inf)))
        ms = [jnp.max(m, axis=1, keepdims=True) for m in ms]

        def v_step(c, carry):
            slot, ls, accs = carry

            @pl.when(c + _AHEAD < _NC)
            def _():
                start_slab(vs, j, c + _AHEAD, prev_slot(slot))

            @pl.when(c + _AHEAD >= _NC)
            def _():
                @pl.when(j < _NJ - 1)
                def _():
                    start_slab(ks, j + 1, c + _AHEAD - _NC, prev_slot(slot))

                @pl.when(j == _NJ - 1)
                def _():
                    @pl.loop(0, _NU_SLAB)
                    def _(u):
                        start_wo((c + _AHEAD - _NC) * _NU_SLAB + u)

            _wait_filled(ring.at[slot], ring_sem.at[slot])
            new_ls, new_accs = [], []
            for b in range(2):
                p = jnp.exp(s_buf[c, b] - ms[b])
                p16 = p.astype(bf16)
                o = _own_rows([
                    jnp.dot(p16, ring[slot, b, r], preferred_element_type=f32)
                    for r in range(_G)])
                new_ls.append(ls[b] + _fold_lanes(jnp.add, p))
                new_accs.append(accs[b] + o)
            return next_slot(slot), tuple(new_ls), tuple(new_accs)

        zero = jnp.zeros((_G, _DH), f32)
        slot, ls, accs = lax.fori_loop(0, _NC, v_step, (slot, (zero, zero), (zero, zero)))
        for b in range(2):
            o_buf[b, j] = accs[b] / jnp.sum(ls[b], axis=1, keepdims=True)
        return slot

    lax.fori_loop(0, _NJ, head_group, 0)

    for b in range(2):
        groups = [o_buf[b, j] for j in range(_NJ)]
        for c in range(4):
            o_buf[b, c] = jnp.concatenate([o[:, 32 * c:32 * c + 32] for o in groups], axis=1)

    def o_row(b, n):
        return o_buf[b, n & 3, pl.ds(n >> 2, 1), :]

    def wait_unit(b, n):
        _wait_filled(wo_buf.at[b, n], wo_sem.at[b * _NU + n])

    def unit(b, n):
        o = jnp.broadcast_to(o_row(b, n), (_G, _DH)).astype(bf16)
        w = jnp.concatenate([wo_buf[b, n, 0], wo_buf[b, n, 1]], axis=0)
        return jnp.dot(o, w, preferred_element_type=f32)

    def first_step(n, acc_a):
        o = o_row(1, n + _NU - _LEAD).astype(bf16).astype(f32)
        wait_unit(0, n)
        col_buf[n] = jnp.broadcast_to(o, (_DH, _DH)).T
        return acc_a + unit(0, n)

    def both_step(n, accs):
        @pl.when(n + _AHEAD * _NU_SLAB < _NU)
        def _():
            start_wo(n + _AHEAD * _NU_SLAB)

        wait_unit(0, n + _LEAD)
        wait_unit(1, n)
        return accs[0] + unit(0, n + _LEAD), accs[1] + unit(1, n)

    def last_step(v, acc):
        n = v + _NU - _LEAD
        for k in range(4):
            wo_copy(1, n, k).wait()
            parts = []
            for half in range(2):
                col = col_buf[v, pl.ds(half * 64 + wo_rows(k), 16)]
                w = wo_buf[1, n, half, pl.ds(wo_rows(k), 16)].astype(f32)
                prod = w * jnp.concatenate([col] * (_D // _DH), axis=1)
                parts.append(prod[:8] + prod[8:])
            acc = acc + (parts[0] + parts[1])
        return acc

    zero = jnp.zeros((_G, _D), f32)
    acc_a = lax.fori_loop(0, _LEAD, first_step, zero)
    acc_a, acc_b = lax.fori_loop(0, _NU - _LEAD, both_step, (acc_a, zero))
    out_ref[0, :, pl.ds(0, _D)] = acc_a[0:1].astype(out_ref.dtype)
    acc_b = jnp.where(lax.broadcasted_iota(jnp.int32, (_G, _D), 0) == 0, acc_b, 0.0)
    acc_b = lax.fori_loop(0, _LEAD, last_step, acc_b)
    out_ref[0, :, pl.ds(_D, _D)] = jnp.sum(acc_b, axis=0, keepdims=True).astype(out_ref.dtype)


def _kernel(*refs):
    pl.run_scoped(
        functools.partial(_body, *refs),
        pltpu.SemaphoreType.DMA((2,)),
        pltpu.SemaphoreType.DMA(()),
        pltpu.SemaphoreType.DMA((_SLOTS,)),
        pltpu.SemaphoreType.DMA((2 * _NU + 3 * _LEAD,)),
    )


@jax.jit
def pallas_concat_heads__mha_block_cached__gqa_block_cached__decode_kernel(
    A_x: jax.Array,
    A_k_cache: jax.Array,
    A_v_cache: jax.Array,
    A_wq: jax.Array,
    A_wo: jax.Array,
    B_x: jax.Array,
    B_k_cache: jax.Array,
    B_v_cache: jax.Array,
    B_wq: jax.Array,
    B_wo: jax.Array,
):
    f32, bf16 = jnp.float32, jnp.bfloat16

    def heads(cache):
        return cache.reshape(_H, _SK, _DH)

    def quarters(w):
        return w.reshape(2, 2, w.shape[0] // 4, w.shape[1])

    return pl.pallas_call(
        _kernel,
        in_specs=[pl.BlockSpec(memory_space=pltpu.HBM)] * 10,
        out_specs=pl.BlockSpec(memory_space=pltpu.VMEM),
        out_shape=jax.ShapeDtypeStruct((1, 1, 2 * _D), A_x.dtype),
        scratch_shapes=[
            pltpu.VMEM((2, 1, 1, _D), bf16),
            pltpu.VMEM((2, _NJ, 2, 2, _D // 4, _G * _DH), bf16),
            pltpu.VMEM((_SLOTS, 2, _G, _T, _DH), bf16),
            pltpu.VMEM((2, _NU, 2, 64, _D), bf16),
            pltpu.VMEM((_NC, 2, _G, _T), f32),
            pltpu.VMEM((2, _NJ, _G, _DH), f32),
            pltpu.VMEM((_LEAD, _DH, _DH), f32),
        ],
        compiler_params=pltpu.CompilerParams(vmem_limit_bytes=48 * 1024 * 1024),
    )(A_x, heads(A_k_cache), heads(A_v_cache), quarters(A_wq), quarters(A_wo),
      B_x, heads(B_k_cache), heads(B_v_cache), quarters(B_wq), quarters(B_wo))
```
